```python
import os as _os
_os.environ.setdefault("JAX_PLATFORMS", "cpu")
import jax
import jax.numpy as jnp

def _softmax(x, axis=-1):
    return jax.nn.softmax(x, axis=axis)
def _gelu(x):
    return jax.nn.gelu(x, approximate=True)
def _silu(x):
    return jax.nn.silu(x)
def _sigmoid(x):
    return jax.nn.sigmoid(x)
def _layernorm(x, axis=-1, eps=1e-5):
    m = jnp.mean(x, axis=axis, keepdims=True)
    v = jnp.var(x, axis=axis, keepdims=True)
    return (x - m) / jnp.sqrt(v + eps)
def _scatter_add(tgt, idx, src, axis=0):
    return tgt.at[idx].add(src)
def _segment_sum(src, seg, n):
    return jax.ops.segment_sum(src, seg, n)
class _Rng:
    def __init__(self, key):
        self._k = key
    def _next(self):
        self._k, sub = jax.random.split(self._k)
        return sub
    def normal(self, shape):
        return jax.random.normal(self._next(), shape, dtype=jnp.bfloat16)
    def randint(self, lo, hi, shape):
        return jax.random.randint(self._next(), shape, lo, hi, dtype=jnp.int32)
    def uniform(self, shape, lo=0.0, hi=1.0):
        return jax.random.uniform(self._next(), shape, jnp.bfloat16, lo, hi)
    def permutation(self, n):
        return jax.random.permutation(self._next(), n)


kernel_name = 'standalone__sliding_block_cached__sampling'

def setup_inputs():
    _rng = _Rng(jax.random.key(int.from_bytes(__import__("os").urandom(4), "little")))
    _w = (lambda a: (lambda t: t.astype(jnp.bfloat16) if jnp.issubdtype(t.dtype, jnp.floating) else t)(jnp.asarray(a)))
    B, Sq, D = 8, 4, 640
    Hq, Hkv, Sk, Dh = 32, 32, 4096, 192
    assert Hq % Hkv == 0, (Hq, Hkv)
    return {
        "x": _w((lambda *s: _rng.normal(s) * 0.8)(B, Sq, D)),
        "k_cache": _w((lambda *s: _rng.normal(s) * 0.8)(B, Hkv, Sk, Dh)),
        "v_cache": _w((lambda *s: _rng.normal(s) * 0.05)(B, Hkv, Sk, Dh)),
        "wq": _w((lambda *s: _rng.normal(s) * 0.8)(D, Hq * Dh) * (D ** -0.5)),
        "wo": _w((lambda *s: _rng.normal(s) * 0.05)(Hq * Dh, D) * ((Hq * Dh) ** -0.5)),
    }

def reference(x, k_cache, v_cache, wq, wo):
    B, Sq, D = x.shape
    Hq, Dh = 32, 192
    Hkv, Sk = k_cache.shape[1], k_cache.shape[2]
    W = min(4096, max(256, Sk // 4))
    rep = Hq // Hkv
    q = (lambda x, *d: x.transpose(*d))((x @ wq).reshape(B, Sq, Hq, Dh), 0, 2, 1, 3)
    k = jnp.repeat(k_cache[:, :, Sk - W:, :], rep, axis=1)
    v = jnp.repeat(v_cache[:, :, Sk - W:, :], rep, axis=1)
    scores = jnp.einsum("bhqd,bhkd->bhqk", q, k) * (Dh ** -0.5)
    p = _softmax(scores, axis=-1)
    o = jnp.einsum("bhqk,bhkd->bhqd", p, v)
    return (lambda x, *d: x.transpose(*d))(o, 0, 2, 1, 3).reshape(B, Sq, Hq * Dh) @ wo
```

```python
import jax
import jax.numpy as jnp
import jax.experimental.pallas as pl
import jax.experimental.pallas.tpu as pltpu

_HQ = 32
_DH = 192
_NBUF = 6
_CW = 256


@jax.jit
def pallas_standalone__sliding_block_cached__sampling_kernel(
    x: jax.Array,
    k_cache: jax.Array,
    v_cache: jax.Array,
    wq: jax.Array,
    wo: jax.Array,
):
    B, Sq, D = x.shape
    Hkv, Sk = k_cache.shape[1], k_cache.shape[2]
    W = min(4096, max(256, Sk // 4))
    assert Hkv == _HQ and Sq == 4 and W % _CW == 0 and (Sk - W) % 128 == 0
    HP = _HQ // 2
    R = 2 * Sq
    C = 2 * _DH
    nsteps = HP * B
    scale = _DH ** -0.5

    def kern(x_hbm, k_hbm, v_hbm, wq_hbm, wo_hbm, o_ref,
             xbuf, xpad, kbuf, vbuf, wqbuf, wobuf, qs, os_, acc,
             ksem, vsem, qsem, osem, xsem):

        def kv_start(i, slot):
            b, h0 = i % B, (i // B) * 2
            nc = W // _CW
            for h in range(2):
                for c in range(nc):
                    for a, (src, dst, sem) in enumerate(
                            ((k_hbm, kbuf, ksem), (v_hbm, vbuf, vsem))):
                        c0 = ((c + 2 * a) % nc) * _CW
                        pltpu.make_async_copy(
                            src.at[b, h0 + h, :, pl.ds(Sk - W + c0, _CW)],
                            dst.at[slot, h, :, pl.ds(c0, _CW)],
                            sem.at[slot]).start(priority=a)

        def slot_wait(buf, sem, slot):
            pltpu.make_async_copy(buf.at[slot], buf.at[slot], sem.at[slot]).wait()

        def qcopy(hp, slot):
            return pltpu.make_async_copy(
                wq_hbm.at[:, pl.ds(pl.multiple_of(hp * C, 128), C)],
                wqbuf.at[slot], qsem.at[slot])

        def ocopy(hp, slot):
            return pltpu.make_async_copy(
                wo_hbm.at[pl.ds(pl.multiple_of(hp * C, 128), C), :],
                wobuf.at[slot], osem.at[slot])

        xcopy = pltpu.make_async_copy(x_hbm, xbuf, xsem)

        xcopy.start()
        qcopy(0, 0).start()
        for i in range(_NBUF):
            kv_start(i, i)
        ocopy(0, 0).start()
        qcopy(1, 1).start()
        ocopy(1, 1).start()

        xcopy.wait()
        for b in range(B):
            xb = xbuf[b].astype(jnp.float32)
            xpad[pl.ds(b * R, Sq), :] = xb
            xpad[pl.ds(b * R + Sq, Sq), :] = xb
        acc[...] = jnp.zeros_like(acc)

        def diag_mask(rows):
            r = jax.lax.broadcasted_iota(jnp.int32, (rows, C), 0)
            c = jax.lax.broadcasted_iota(jnp.int32, (rows, C), 1)
            return ((r % R) < Sq) == (c < _DH)

        def body(i, _):
            slot = i % _NBUF
            b = i % B
            hp = i // B
            wslot = hp % 2

            @pl.when(b == 0)
            def _():
                qcopy(hp, wslot).wait()
                q = jnp.dot(xpad[...].astype(jnp.bfloat16), wqbuf[wslot],
                            preferred_element_type=jnp.float32)
                qs[...] = jnp.where(diag_mask(B * R), q, 0.0)

                @pl.when(hp + 2 < HP)
                def _():
                    qcopy(hp + 2, wslot).start(priority=0)

            row = pl.multiple_of(b * R, R)
            q = qs[pl.ds(row, R), :].astype(jnp.bfloat16)
            slot_wait(kbuf, ksem, slot)
            kt = kbuf[slot].reshape(C, W)
            s = jnp.dot(q, kt, preferred_element_type=jnp.float32) * scale
            m = jnp.max(s, axis=-1, keepdims=True)
            p = jnp.exp(s - m)
            l = jnp.sum(p, axis=-1, keepdims=True)
            slot_wait(vbuf, vsem, slot)
            vt = vbuf[slot].reshape(C, W)
            o = jax.lax.dot_general(
                p.astype(jnp.bfloat16), vt, (((1,), (1,)), ((), ())),
                preferred_element_type=jnp.float32)
            os_[pl.ds(row, R), :] = jnp.where(diag_mask(R), o / l, 0.0)

            @pl.when(i + _NBUF < nsteps)
            def _():
                kv_start(i + _NBUF, slot)

            @pl.when(b == B - 1)
            def _():
                ocopy(hp, wslot).wait()
                acc[...] += jnp.dot(os_[...].astype(jnp.bfloat16), wobuf[wslot],
                                    preferred_element_type=jnp.float32)

                @pl.when(hp + 2 < HP)
                def _():
                    ocopy(hp + 2, wslot).start(priority=1)

            return None

        jax.lax.fori_loop(0, nsteps, body, None)
        for b in range(B):
            o_ref[b] = (acc[pl.ds(b * R, Sq), :]
                        + acc[pl.ds(b * R + Sq, Sq), :]).astype(o_ref.dtype)

    hbm = pl.BlockSpec(memory_space=pl.ANY)
    return pl.pallas_call(
        kern,
        out_shape=jax.ShapeDtypeStruct(x.shape, x.dtype),
        in_specs=[hbm] * 5,
        out_specs=pl.BlockSpec(memory_space=pltpu.VMEM),
        scratch_shapes=[
            pltpu.VMEM((B, Sq, D), x.dtype),
            pltpu.VMEM((B * R, D), jnp.float32),
            pltpu.VMEM((_NBUF, 2, _DH, W), k_cache.dtype),
            pltpu.VMEM((_NBUF, 2, _DH, W), v_cache.dtype),
            pltpu.VMEM((2, D, C), wq.dtype),
            pltpu.VMEM((2, C, D), wo.dtype),
            pltpu.VMEM((B * R, C), jnp.float32),
            pltpu.VMEM((B * R, C), jnp.float32),
            pltpu.VMEM((B * R, D), jnp.float32),
            pltpu.SemaphoreType.DMA((_NBUF,)),
            pltpu.SemaphoreType.DMA((_NBUF,)),
            pltpu.SemaphoreType.DMA((2,)),
            pltpu.SemaphoreType.DMA((2,)),
            pltpu.SemaphoreType.DMA(()),
        ],
        compiler_params=pltpu.CompilerParams(
            vmem_limit_bytes=100 * 1024 * 1024, disable_bounds_checks=True),
    )(x, jnp.swapaxes(k_cache, 2, 3), jnp.swapaxes(v_cache, 2, 3), wq, wo)
```

```python
import jax
import jax.numpy as jnp
import jax.experimental.pallas as pl
import jax.experimental.pallas.tpu as pltpu

_HQ = 32
_DH = 192
_G = 4
_NBUF = 3
_RUN = 512
_KV_STRIDE = 32
_WQ_STRIDE = 16
_WO_ROWS = 32
_KV_MUL, _WQ_MUL, _WO_MUL = 15, 41, 65


@jax.jit
def pallas_standalone__sliding_block_cached__sampling_kernel(
    x: jax.Array,
    k_cache: jax.Array,
    v_cache: jax.Array,
    wq: jax.Array,
    wo: jax.Array,
):
    B, Sq, D = x.shape
    Hkv, Sk = k_cache.shape[1], k_cache.shape[2]
    W = min(4096, max(256, Sk // 4))
    assert Hkv == _HQ and (B, Sq) == (8, 4)
    assert W % _RUN == 0 and Sk % 128 == 0 and D % (8 * _WQ_STRIDE) == 0
    E = _HQ * _DH
    HG = _HQ // _G
    C = _G * _DH
    nsteps = HG * B
    scale = _DH ** -0.5
    kv_runs = C // (8 * _KV_STRIDE)
    wq_runs = D // (8 * _WQ_STRIDE)
    kv_pieces = [((n * _KV_MUL) % _KV_STRIDE, c)
                 for n in range(_KV_STRIDE) for c in range(0, W, _RUN)]
    n_kv = len(kv_pieces)
    n_wq = _WQ_STRIDE * (E // _RUN)
    n_late = C // _WO_ROWS
    n_early = E // _WO_ROWS - n_late
    assert n_wq == n_early + n_late and n_late <= n_kv

    def kern(x_hbm, k_hbm, v_hbm, wq_hbm, wo_hbm, o_ref,
             xbuf, xpad, kv, wqbuf, wobuf, qs, os_, acc,
             kv_sem, x_sem, wq_sem, wo_sem):

        def kv_start(a, i, n):
            j, c = kv_pieces[n]
            slot = i % _NBUF
            pltpu.make_async_copy(
                (k_hbm, v_hbm)[a].at[i % B, i // B, :, j, :,
                                     pl.ds(Sk - W + c, _RUN)],
                kv.at[slot, a, :, j, :, pl.ds(c, _RUN)],
                kv_sem.at[slot]).start(priority=a)

        def wq_start(n):
            n = (n * _WQ_MUL) % n_wq
            j = n % _WQ_STRIDE
            cols = pl.ds(pl.multiple_of((n // _WQ_STRIDE) * _RUN, _RUN), _RUN)
            pltpu.make_async_copy(wq_hbm.at[:, j, :, cols], wqbuf.at[:, j, :, cols],
                                  wq_sem).start(priority=0)

        def wo_start(n):
            rows = pl.ds(pl.multiple_of(n * _WO_ROWS, _WO_ROWS), _WO_ROWS)
            pltpu.make_async_copy(wo_hbm.at[rows], wobuf.at[rows],
                                  wo_sem).start(priority=1)

        def wait_all(ref, sem):
            pltpu.make_async_copy(ref, ref, sem).wait()

        def issue(i, last=False):
            for n in range(n_kv):
                kv_start(0, i, n)
                m = n + n_late
                if m < n_kv:
                    kv_start(1, i, m)
                elif last:
                    wo_start(n_early + m - n_kv)
                else:
                    kv_start(1, i + 1, m - n_kv)

        xcopy = pltpu.make_async_copy(x_hbm, xbuf, x_sem)
        xcopy.start()

        @pl.loop(0, n_early)
        def _(n):
            wq_start(n)
            wo_start((n * _WO_MUL) % n_early)

        for n in range(n_late):
            wq_start(n_early + n)
            kv_start(1, 0, n)

        @pl.loop(0, _NBUF - 1)
        def _(i):
            issue(i)

        acc[...] = jnp.zeros_like(acc)
        os_[...] = jnp.zeros_like(os_)
        xcopy.wait()
        wait_all(wqbuf, wq_sem)
        wait_all(wobuf.at[pl.ds(0, n_early * _WO_ROWS)], wo_sem)
        for b in range(B):
            xb = xbuf[b].astype(jnp.float32)
            xpad[pl.ds(b * 8, Sq), :] = xb
            xpad[pl.ds(b * 8 + Sq, Sq), :] = xb

        def head_mask(h):
            r = jax.lax.broadcasted_iota(jnp.int32, (8, C), 0)
            c = jax.lax.broadcasted_iota(jnp.int32, (8, C), 1)
            lo = jnp.where(r < Sq, h * _DH, (h + 1) * _DH)
            return (c >= lo) & (c < lo + _DH)

        @pl.loop(0, nsteps)
        def _(i):
            b = i % B
            slot = i % _NBUF
            cols = pl.ds(pl.multiple_of((i // B) * C, 128), C)
            wait_all(kv.at[slot], kv_sem.at[slot])

            @pl.when(b == 0)
            def _():
                w = wqbuf[:, :, :, cols].reshape(D, C)
                qs[...] = jnp.dot(xpad[...].astype(w.dtype), w,
                                  preferred_element_type=jnp.float32)

            m0, m1 = head_mask(0), head_mask(2)
            q8 = qs[pl.ds(pl.multiple_of(b * 8, 8), 8), :]
            q = jnp.concatenate(
                [jnp.where(m0, q8, 0.0), jnp.where(m1, q8, 0.0)], axis=0)
            kt = kv[slot, 0].reshape(C, W)
            s = jnp.dot(q.astype(kt.dtype), kt,
                        preferred_element_type=jnp.float32) * scale
            p = jnp.exp(s - jnp.max(s, axis=-1, keepdims=True))
            l = jnp.sum(p, axis=-1, keepdims=True)
            vt = kv[slot, 1].reshape(C, W)
            o = jax.lax.dot_general(
                p.astype(vt.dtype), vt, (((1,), (1,)), ((), ())),
                preferred_element_type=jnp.float32) / l
            o = jnp.where(m0, o[0:8], jnp.where(m1, o[8:16], 0.0))
            o = o + pltpu.roll(o, Sq, 0)
            rows = pl.ds(pl.multiple_of((b // 2) * 8, 8), 8)
            half = jax.lax.broadcasted_iota(jnp.int32, (8, C), 0) // Sq
            os_[rows, :] = jnp.where(half == b % 2, o, os_[rows, :])

            nxt = i + (_NBUF - 1)

            @pl.when(nxt < nsteps - 1)
            def _():
                issue(nxt)

            @pl.when(nxt == nsteps - 1)
            def _():
                issue(nsteps - 1, last=True)

            @pl.when((b == B - 1) & (i < nsteps - 1))
            def _():
                acc[...] += jnp.dot(os_[...].astype(wobuf.dtype), wobuf[cols, :],
                                    preferred_element_type=jnp.float32)

        rows = pl.ds(n_early * _WO_ROWS, C)
        ob = os_[...].astype(wobuf.dtype)
        wait_all(wobuf.at[rows], wo_sem)
        out = acc[...] + jnp.dot(ob, wobuf[rows, :],
                                 preferred_element_type=jnp.float32)
        for b in range(B):
            o_ref[b] = out[b * Sq:(b + 1) * Sq, :].astype(o_ref.dtype)

    kv_view = (B, HG, kv_runs, _KV_STRIDE, 8, Sk)
    wq_view = (wq_runs, _WQ_STRIDE, 8, E)
    hbm = pl.BlockSpec(memory_space=pl.ANY)
    return pl.pallas_call(
        kern,
        out_shape=jax.ShapeDtypeStruct(x.shape, x.dtype),
        in_specs=[hbm] * 5,
        out_specs=pl.BlockSpec(memory_space=pltpu.VMEM),
        scratch_shapes=[
            pltpu.VMEM((B, Sq, D), x.dtype),
            pltpu.VMEM((B * 8, D), jnp.float32),
            pltpu.VMEM((_NBUF, 2, kv_runs, _KV_STRIDE, 8, W),
                       k_cache.dtype),
            pltpu.VMEM(wq_view, wq.dtype),
            pltpu.VMEM((E, D), wo.dtype),
            pltpu.VMEM((B * 8, C), jnp.float32),
            pltpu.VMEM((B * Sq, C), jnp.float32),
            pltpu.VMEM((B * Sq, D), jnp.float32),
            pltpu.SemaphoreType.DMA((_NBUF,)),
            pltpu.SemaphoreType.DMA(()),
            pltpu.SemaphoreType.DMA(()),
            pltpu.SemaphoreType.DMA(()),
        ],
        compiler_params=pltpu.CompilerParams(vmem_limit_bytes=64 * 1024 * 1024),
    )(x,
      jnp.swapaxes(k_cache, 2, 3).reshape(kv_view),
      jnp.swapaxes(v_cache, 2, 3).reshape(kv_view),
      wq.reshape(wq_view),
      wo)
```
